```python
import os as _os
_os.environ.setdefault('JAX_PLATFORMS', 'cpu')
import jax
import jax.numpy as jnp

def _softmax(x, axis=-1):
    return jax.nn.softmax(x, axis=axis)

def _gelu(x):
    return jax.nn.gelu(x, approximate=True)

def _silu(x):
    return jax.nn.silu(x)

def _sigmoid(x):
    return jax.nn.sigmoid(x)

def _layernorm(x, axis=-1, eps=1e-05):
    m = jnp.mean(x, axis=axis, keepdims=True)
    v = jnp.var(x, axis=axis, keepdims=True)
    return (x - m) / jnp.sqrt(v + eps)

def _scatter_add(tgt, idx, src, axis=0):
    return tgt.at[idx].add(src)

def _segment_sum(src, seg, n):
    return jax.ops.segment_sum(src, seg, n)

class _Rng:

    def __init__(self, key):
        self._k = key

    def _next(self):
        self._k, sub = jax.random.split(self._k)
        return sub

    def normal(self, shape):
        return jax.random.normal(self._next(), shape, dtype=jnp.bfloat16)

    def randint(self, lo, hi, shape):
        return jax.random.randint(self._next(), shape, lo, hi, dtype=jnp.int32)

    def uniform(self, shape, lo=0.0, hi=1.0):
        return jax.random.uniform(self._next(), shape, jnp.bfloat16, lo, hi)

    def permutation(self, n):
        return jax.random.permutation(self._next(), n)
kernel_name = 'standalone__conformer_family_e_branchformer__speech'

def setup_inputs():
    _rng = _Rng(jax.random.key(int.from_bytes(__import__("os").urandom(4), "little")))
    _w = lambda a: (lambda t: t.astype(jnp.bfloat16) if jnp.issubdtype(t.dtype, jnp.floating) else t)(jnp.asarray(a))
    B, T, D, K = (2, 4000, 512, 5)
    return {'x': _w((lambda *s: _rng.normal(s) * 0.05)(B, T, D)), 'w_qkv': _w((lambda *s: _rng.normal(s) * 0.05)(D, 3 * D)), 'w_att_out': _w((lambda *s: _rng.normal(s) * 0.05)(D, D)), 'w_mlp_in': _w((lambda *s: _rng.normal(s) * 0.05)(D, 2 * D)), 'dw_csgu': _w((lambda *s: _rng.normal(s) * 0.05)(K, D)), 'w_mlp_out': _w((lambda *s: _rng.normal(s) * 0.05)(D, D)), 'dw_merge': _w((lambda *s: _rng.normal(s) * 0.05)(K, 2 * D)), 'w_merge': _w((lambda *s: _rng.normal(s) * 0.05)(2 * D, D))}

def reference(x, w_qkv, w_att_out, w_mlp_in, dw_csgu, w_mlp_out, dw_merge, w_merge):
    B, T, D = x.shape
    K = dw_csgu.shape[0]
    pad = K // 2
    xa = _layernorm(x, axis=-1)
    qkv = jnp.einsum('btd,de->bte', xa, w_qkv)
    q, k, v = (qkv[..., :D].copy(), qkv[..., D:2 * D].copy(), qkv[..., 2 * D:].copy())
    scores = jnp.einsum('btd,bsd->bts', q, k) * D ** (-0.5)
    p = _softmax(scores, axis=-1)
    attn = jnp.einsum('bts,bsd->btd', p, v)
    glob = jnp.einsum('btd,de->bte', attn, w_att_out)
    xc = _layernorm(x, axis=-1)
    h = _gelu(jnp.einsum('btd,de->bte', xc, w_mlp_in))
    u, g = (h[..., :D].copy(), h[..., D:].copy())
    g = _layernorm(g, axis=-1)
    gp = jnp.pad(g, ((0, 0), (pad, pad), (0, 0)))
    gc = jnp.zeros_like(g)
    for i in range(K):
        gc = gc + gp[:, i:i + T, :] * dw_csgu[i][None, None, :]
    loc = jnp.einsum('btd,de->bte', u * gc, w_mlp_out)
    m = jnp.concatenate([glob, loc], axis=-1)
    mp = jnp.pad(m, ((0, 0), (pad, pad), (0, 0)))
    mc = jnp.zeros_like(m)
    for i in range(K):
        mc = mc + mp[:, i:i + T, :] * dw_merge[i][None, None, :]
    m = m + mc
    return x + jnp.einsum('btc,cd->btd', m, w_merge)
```

```python
import functools
import math

import jax
import jax.numpy as jnp
from jax import lax
import jax.experimental.pallas as pl
import jax.experimental.pallas.tpu as pltpu

F32 = jnp.float32
BF16 = jnp.bfloat16
LANES = 128
PAD = 8
EPS = 1e-5


def _dot(a, b):
    return jnp.dot(a, b, preferred_element_type=F32)


def _dot_nt(a, b):
    return lax.dot_general(a, b, (((1,), (1,)), ((), ())),
                           preferred_element_type=F32)


def _layernorm(v):
    mu = jnp.mean(v, axis=-1, keepdims=True)
    c = v - mu
    var = jnp.mean(c * c, axis=-1, keepdims=True)
    return c * lax.rsqrt(var + EPS)


def _gelu(v):
    c0 = math.sqrt(2.0 / math.pi)
    inner = v * (c0 + (c0 * 0.044715) * (v * v))
    half = 0.5 * v
    return half + half * jnp.tanh(inner)


def _make_kernel(T, D, TQ, K, CK):
    NT = T // TQ
    NC = D // LANES
    HALF = K // 2
    chunks = [(c0, min(CK, T - c0)) for c0 in range(0, T, CK)]
    qk_scale = (D ** -0.5) * math.log2(math.e)

    def kernel(x_ref, wqkv_ref, wao_ref, win_ref, dwc_ref, wout_ref, dwm_ref,
               wmg_ref, o_ref,
               wqk_s, wvo_s, xa_s, xv_s, q_s, u_s, gn_s, m_s):
        b = pl.program_id(0)
        s = pl.program_id(1)

        @pl.when(jnp.logical_and(b == 0, s == 0))
        def _init():
            wqk = _dot_nt(wqkv_ref[:, 0:D], wqkv_ref[:, D:2 * D]) * qk_scale
            wqk_s[...] = wqk.astype(BF16)
            wvo = _dot(wqkv_ref[:, 2 * D:3 * D], wao_ref[...])
            wvo_s[...] = (wvo - wvo[D - 1:D, :]).astype(BF16)
            zrow = jnp.zeros((PAD, LANES), F32)
            for c in range(NC):
                gn_s[c, 0:PAD, :] = zrow
                gn_s[c, PAD + T:PAD + T + PAD, :] = zrow
            for c in range(2 * NC):
                m_s[c, 0:PAD, :] = zrow
                m_s[c, PAD + T:PAD + T + PAD, :] = zrow

        def phase1(j):
            r0 = pl.multiple_of(j * TQ, 16)
            xa = _layernorm(x_ref[0].astype(F32)).astype(BF16)
            xa_s[pl.ds(r0, TQ), :] = xa
            lane = lax.broadcasted_iota(jnp.int32, (TQ, D), 1)
            xv_s[pl.ds(r0, TQ), :] = jnp.where(lane == D - 1,
                                               jnp.ones_like(xa), xa)
            g = _layernorm(_gelu(_dot(xa, win_ref[:, D:2 * D])))
            for c in range(NC):
                gn_s[c, pl.ds(PAD + r0, TQ), :] = g[:, c * LANES:(c + 1) * LANES]
            u_s[pl.ds(r0, TQ), :] = _gelu(_dot(xa, win_ref[:, 0:D]))
            q_s[pl.ds(r0, TQ), :] = _dot(xa, wqk_s[...]).astype(BF16)

        def conv(src, nct, dw, r0):
            outs = []
            for c in range(nct):
                acc = None
                for k in range(K):
                    t = (src[c, pl.ds(r0 + (PAD - HALF + k), TQ), :]
                         * dw[k:k + 1, c * LANES:(c + 1) * LANES])
                    acc = t if acc is None else acc + t
                outs.append(acc)
            return jnp.concatenate(outs, axis=1)

        def attend(i):
            r0 = pl.multiple_of(i * TQ, 16)
            q = q_s[pl.ds(r0, TQ), :]
            ss = []
            mrun = None
            for c0, cw in chunks:
                sc = _dot_nt(q, xa_s[c0:c0 + cw, :])
                ss.append(sc)
                nfull = cw // LANES
                for t in range(nfull):
                    st = sc[:, t * LANES:(t + 1) * LANES]
                    mrun = st if mrun is None else jnp.maximum(mrun, st)
                if cw % LANES:
                    mtail = jnp.max(sc[:, nfull * LANES:], axis=1, keepdims=True)
                    mrun = jnp.maximum(mrun, mtail)
            m = jnp.max(mrun, axis=1, keepdims=True)
            acc = None
            for (c0, cw), sc in zip(chunks, ss):
                p = jnp.exp2(sc - m).astype(BF16)
                o = _dot(p, xv_s[c0:c0 + cw, :])
                acc = o if acc is None else acc + o
            on = (acc * (1.0 / acc[:, D - 1:D])).astype(BF16)
            glob = _dot(on, wvo_s[...])
            for c in range(NC):
                m_s[c, pl.ds(PAD + r0, TQ), :] = glob[:, c * LANES:(c + 1) * LANES]
            gc = conv(gn_s, NC, dwc_ref[...].astype(F32), r0)
            t = (u_s[pl.ds(r0, TQ), :] * gc).astype(BF16)
            loc = _dot(t, wout_ref[...])
            for c in range(NC):
                m_s[NC + c, pl.ds(PAD + r0, TQ), :] = loc[:, c * LANES:(c + 1) * LANES]

        def merge(i):
            r0 = pl.multiple_of(i * TQ, 16)
            dw = dwm_ref[...].astype(F32)
            row = lax.broadcasted_iota(jnp.int32, dw.shape, 0)
            dw = jnp.where(row == HALF, dw + 1.0, dw)
            mm = conv(m_s, 2 * NC, dw, r0).astype(BF16)
            y = _dot(mm, wmg_ref[...])
            o_ref[0] = (x_ref[0].astype(F32) + y).astype(o_ref.dtype)

        @pl.when(s < NT)
        def _():
            phase1(s)

        @pl.when(s == NT)
        def _():
            attend(0)

        @pl.when(jnp.logical_and(s > NT, s < 2 * NT))
        def _():
            attend(s - NT)
            merge(s - NT - 1)

        @pl.when(s == 2 * NT)
        def _():
            merge(NT - 1)

    return kernel


@jax.jit
def pallas_standalone__conformer_family_e_branchformer__speech_kernel(
    x, w_qkv, w_att_out, w_mlp_in, dw_csgu, w_mlp_out, dw_merge, w_merge,
):
    B, T, D = x.shape
    K = dw_csgu.shape[0]
    TQ = 400
    CK = 512
    NT = T // TQ
    NC = D // LANES

    def x_map(b, s):
        return (b, jnp.where(s < NT, s, jnp.clip(s - NT - 1, 0, NT - 1)), 0)

    def o_map(b, s):
        return (b, jnp.clip(s - NT - 1, 0, NT - 1), 0)

    def full(a):
        return pl.BlockSpec(a.shape, lambda b, s: (0,) * a.ndim,
                            pipeline_mode=pl.Buffered(1))

    return pl.pallas_call(
        _make_kernel(T, D, TQ, K, CK),
        grid=(B, 2 * NT + 1),
        in_specs=[pl.BlockSpec((1, TQ, D), x_map),
                  full(w_qkv), full(w_att_out), full(w_mlp_in), full(dw_csgu),
                  full(w_mlp_out), full(dw_merge), full(w_merge)],
        out_specs=pl.BlockSpec((1, TQ, D), o_map),
        out_shape=jax.ShapeDtypeStruct((B, T, D), x.dtype),
        scratch_shapes=[
            pltpu.VMEM((D, D), BF16),
            pltpu.VMEM((D, D), BF16),
            pltpu.VMEM((T, D), BF16),
            pltpu.VMEM((T, D), BF16),
            pltpu.VMEM((T, D), BF16),
            pltpu.VMEM((T, D), F32),
            pltpu.VMEM((NC, T + 2 * PAD, LANES), F32),
            pltpu.VMEM((2 * NC, T + 2 * PAD, LANES), F32),
        ],
        compiler_params=pltpu.CompilerParams(
            dimension_semantics=("arbitrary", "arbitrary"),
            vmem_limit_bytes=110 * 1024 * 1024),
        name="ebranchformer",
    )(x, w_qkv, w_att_out, w_mlp_in, dw_csgu, w_mlp_out, dw_merge, w_merge)
```

```python
import math

import jax
import jax.numpy as jnp
from jax import lax
import jax.experimental.pallas as pl
import jax.experimental.pallas.tpu as pltpu

F32 = jnp.float32
BF16 = jnp.bfloat16
LANES = 128
PAD = 8
EPS = 1e-5


def _dot(a, b):
    return jnp.dot(a, b, preferred_element_type=F32)


def _dot_nt(a, b):
    return lax.dot_general(a, b, (((1,), (1,)), ((), ())),
                           preferred_element_type=F32)


def _layernorm(v):
    mu = jnp.mean(v, axis=-1, keepdims=True)
    c = v - mu
    var = jnp.mean(c * c, axis=-1, keepdims=True)
    return c * lax.rsqrt(var + EPS)


def _gelu(v):
    c0 = math.sqrt(2.0 / math.pi)
    inner = v * (c0 + (c0 * 0.044715) * (v * v))
    half = 0.5 * v
    return half + half * jnp.tanh(inner)


def _rowmax(sc):
    cw = sc.shape[1]
    nfull = cw // LANES
    mr = None
    for t in range(nfull):
        st = sc[:, t * LANES:(t + 1) * LANES]
        mr = st if mr is None else jnp.maximum(mr, st)
    m = jnp.max(mr, axis=1, keepdims=True)
    if cw % LANES:
        m = jnp.maximum(m, jnp.max(sc[:, nfull * LANES:], axis=1, keepdims=True))
    return m


def _make_kernel(B, T, D, TQ, K, CK):
    NT = T // TQ
    NC = D // LANES
    HALF = K // 2
    chunks = [(c0, min(CK, T - c0)) for c0 in range(0, T, CK)]
    NCH = len(chunks)
    qk_scale = (D ** -0.5) * math.log2(math.e)

    def kernel(x_hbm, wqkv_hbm, wao_hbm, win_hbm, dwc_hbm, wout_hbm,
               dwm_hbm, wmg_hbm, o_hbm,
               x_s, wqkv_ref, wao_ref, win_ref, dwc_ref, wout_ref, dwm_ref,
               wmg_ref, o_s,
               wqk_s, wvo_s, xa_s, xv_s, q_s, u_s, gn_s, mg_s, ml_s,
               xsem, wsem, osem):

        def x_copy(b, j):
            rows = pl.ds(pl.multiple_of(j * TQ, 16), TQ)
            return pltpu.make_async_copy(x_hbm.at[b, rows], x_s.at[b, rows],
                                         xsem.at[b * NT + j])

        def w_copy(k, src, dst):
            return pltpu.make_async_copy(src, dst, wsem.at[k])

        cp_wqk = w_copy(0, wqkv_hbm.at[:, 0:2 * D], wqkv_ref.at[:, 0:2 * D])
        cp_win = w_copy(1, win_hbm, win_ref)
        late_copies = [
            w_copy(2, wqkv_hbm.at[:, 2 * D:3 * D], wqkv_ref.at[:, 2 * D:3 * D]),
            w_copy(3, wao_hbm, wao_ref), w_copy(4, dwc_hbm, dwc_ref),
            w_copy(5, wout_hbm, wout_ref), w_copy(6, dwm_hbm, dwm_ref),
            w_copy(7, wmg_hbm, wmg_ref)]

        def o_copy(g):
            b = g // NT
            rows = pl.ds(pl.multiple_of((g % NT) * TQ, 16), TQ)
            slot = g % 2
            return pltpu.make_async_copy(o_s.at[slot], o_hbm.at[b, rows],
                                         osem.at[slot])

        x_copy(0, 0).start()
        cp_wqk.start()

        zrow = jnp.zeros((PAD, LANES), F32)
        for ref in (gn_s, mg_s, ml_s):
            for c in range(NC):
                ref[c, 0:PAD, :] = zrow
                ref[c, PAD + T:PAD + T + PAD, :] = zrow
        zblk = jnp.zeros((2 * TQ + PAD, LANES), F32)
        for ref in (mg_s, ml_s):
            for c in range(NC):
                ref[c, T - 2 * TQ:T + PAD, :] = zblk

        cp_wqk.wait()
        cp_win.start()
        x_copy(0, 1).start()
        wqk = _dot_nt(wqkv_ref[:, 0:D], wqkv_ref[:, D:2 * D]) * qk_scale
        wqk_s[...] = wqk.astype(BF16)

        def fold_vo():
            for cp in late_copies:
                cp.wait()
            wvo = _dot(wqkv_ref[:, 2 * D:3 * D], wao_ref[...])
            wvo_s[...] = (wvo - wvo[D - 1:D, :]).astype(BF16)

        def p1_norm(b, j):
            r0 = pl.multiple_of(j * TQ, 16)
            xa = _layernorm(x_s[b, pl.ds(r0, TQ), :].astype(F32))
            lane = lax.broadcasted_iota(jnp.int32, (TQ, D), 1)
            xv_s[pl.ds(r0, TQ), :] = jnp.where(lane == D - 1, 1.0, xa).astype(BF16)
            xa = xa.astype(BF16)
            xa_s[pl.ds(r0, TQ), :] = xa
            q_s[pl.ds(r0, TQ), :] = _dot(xa, wqk_s[...]).astype(BF16)

        def p1_mlp(j):
            r0 = pl.multiple_of(j * TQ, 16)
            xa = xa_s[pl.ds(r0, TQ), :]
            g = _layernorm(_gelu(_dot(xa, win_ref[:, D:2 * D])))
            for c in range(NC):
                gn_s[c, pl.ds(PAD + r0, TQ), :] = g[:, c * LANES:(c + 1) * LANES]
            u_s[pl.ds(r0, TQ), :] = _gelu(_dot(xa, win_ref[:, 0:D]))

        def conv_col(src, c, dw, r0):
            acc = None
            for k in range(K):
                t = src[c, pl.ds(r0 + (PAD - HALF + k), TQ), :] * dw[k:k + 1, :]
                acc = t if acc is None else acc + t
            return acc

        def block(i, g):
            state = {}
            if i is not None:
                r0 = pl.multiple_of(i * TQ, 16)
                dwc = dwc_ref[...].astype(F32)

                def loc_chunk(c):
                    def f():
                        gc = conv_col(gn_s, c, dwc[:, c * LANES:(c + 1) * LANES], r0)
                        t = (u_s[pl.ds(r0, TQ), c * LANES:(c + 1) * LANES] * gc).astype(BF16)
                        o = _dot(t, wout_ref[c * LANES:(c + 1) * LANES, :])
                        state["loc"] = o if c == 0 else state["loc"] + o
                        if c == NC - 1:
                            for cc in range(NC):
                                ml_s[cc, pl.ds(PAD + r0, TQ), :] = (
                                    state["loc"][:, cc * LANES:(cc + 1) * LANES])
                    return f
                loc_fns = [loc_chunk(c) for c in range(NC)]
            gp = g + NT
            rm = pl.multiple_of(lax.rem(gp, NT) * TQ, 16)
            bm = jnp.maximum(g, 0) // NT
            slot = lax.rem(gp, 2)
            dwm = dwm_ref[...].astype(F32)
            row = lax.broadcasted_iota(jnp.int32, dwm.shape, 0)
            dwm = jnp.where(row == HALF, dwm + 1.0, dwm)

            def mrg_chunk(c):
                def f():
                    src = mg_s if c < NC else ml_s
                    mm = conv_col(src, c % NC, dwm[:, c * LANES:(c + 1) * LANES], rm)
                    o = _dot(mm.astype(BF16), wmg_ref[c * LANES:(c + 1) * LANES, :])
                    state["y"] = o if c == 0 else state["y"] + o
                    if c == 2 * NC - 1:
                        res = x_s[bm, pl.ds(rm, TQ), :].astype(F32) + state["y"]
                        o_s[slot] = res.astype(o_s.dtype)
                return f
            mrg_fns = [mrg_chunk(c) for c in range(2 * NC)]

            if i is None:
                for f in mrg_fns:
                    f()
                return

            slots = [mrg_fns[0:2], mrg_fns[2:4], mrg_fns[4:6], mrg_fns[6:8],
                     [], [], loc_fns[0:2], loc_fns[2:4]]

            q = q_s[pl.ds(r0, TQ), :]

            def qk(idx):
                c0, cw = chunks[idx]
                return _dot_nt(q, xa_s[c0:c0 + cw, :])

            nxt = qk(0)
            acc = None
            m = None
            for idx, (c0, cw) in enumerate(chunks):
                sc = nxt
                if idx + 1 < NCH:
                    nxt = qk(idx + 1)
                mc = _rowmax(sc)
                mn = mc if m is None else jnp.maximum(m, mc)
                p = jnp.exp2(sc - mn).astype(BF16)
                o = _dot(p, xv_s[c0:c0 + cw, :])
                acc = o if acc is None else acc * jnp.exp2(m - mn) + o
                m = mn
                for f in slots[idx]:
                    f()
            on = (acc * (1.0 / acc[:, D - 1:D])).astype(BF16)
            glob = _dot(on, wvo_s[...])
            for c in range(NC):
                mg_s[c, pl.ds(PAD + r0, TQ), :] = glob[:, c * LANES:(c + 1) * LANES]

        def merge_step(i, g):
            @pl.when(g >= 2)
            def _():
                o_copy(g - 2).wait()
            block(i, g)

            @pl.when(g >= 0)
            def _():
                o_copy(g).start()

        def batch_body(b, carry):
            x_copy(b, 0).wait()
            p1_norm(b, 0)
            pl.when(b == 0)(cp_win.wait)

            def p1_body(j, c):
                @pl.when(jnp.logical_and(b == 0, j + 1 < NT))
                def _():
                    x_copy(0, j + 1).start()

                @pl.when(jnp.logical_and(b == 0, j == 2))
                def _():
                    for cp in late_copies:
                        cp.start()
                x_copy(b, j).wait()
                p1_mlp(j - 1)
                p1_norm(b, j)
                return c
            lax.fori_loop(1, NT, p1_body, 0)
            p1_mlp(NT - 1)
            pl.when(b == 0)(fold_vo)

            def att_body(i, c):
                @pl.when(b + 1 < B)
                def _():
                    x_copy(b + 1, i).start()
                merge_step(i, b * NT + i - 2)
                return c
            lax.fori_loop(0, NT, att_body, 0)
            return carry

        lax.fori_loop(0, B, batch_body, 0)

        def tail_body(k, c):
            merge_step(None, B * NT - 2 + k)
            return c
        lax.fori_loop(0, 2, tail_body, 0)
        o_copy(B * NT - 2).wait()
        o_copy(B * NT - 1).wait()

    return kernel


@jax.jit
def pallas_standalone__conformer_family_e_branchformer__speech_kernel(
    x, w_qkv, w_att_out, w_mlp_in, dw_csgu, w_mlp_out, dw_merge, w_merge,
):
    B, T, D = x.shape
    K = dw_csgu.shape[0]
    TQ = 400
    CK = 512
    NT = T // TQ
    NC = D // LANES
    T2 = T + 2 * PAD
    dt = x.dtype
    hbm = pl.BlockSpec(memory_space=pl.ANY)
    return pl.pallas_call(
        _make_kernel(B, T, D, TQ, K, CK),
        in_specs=[hbm] * 8,
        out_specs=hbm,
        out_shape=jax.ShapeDtypeStruct((B, T, D), dt),
        scratch_shapes=[
            pltpu.VMEM((B, T, D), dt),
            pltpu.VMEM(w_qkv.shape, dt),
            pltpu.VMEM(w_att_out.shape, dt),
            pltpu.VMEM(w_mlp_in.shape, dt),
            pltpu.VMEM(dw_csgu.shape, dt),
            pltpu.VMEM(w_mlp_out.shape, dt),
            pltpu.VMEM(dw_merge.shape, dt),
            pltpu.VMEM(w_merge.shape, dt),
            pltpu.VMEM((2, TQ, D), dt),
            pltpu.VMEM((D, D), BF16),
            pltpu.VMEM((D, D), BF16),
            pltpu.VMEM((T, D), BF16),
            pltpu.VMEM((T, D), BF16),
            pltpu.VMEM((T, D), BF16),
            pltpu.VMEM((T, D), F32),
            pltpu.VMEM((NC, T2, LANES), F32),
            pltpu.VMEM((NC, T2, LANES), F32),
            pltpu.VMEM((NC, T2, LANES), F32),
            pltpu.SemaphoreType.DMA((B * NT,)),
            pltpu.SemaphoreType.DMA((8,)),
            pltpu.SemaphoreType.DMA((2,)),
        ],
        compiler_params=pltpu.CompilerParams(
            vmem_limit_bytes=110 * 1024 * 1024),
        name="ebranchformer",
    )(x, w_qkv, w_att_out, w_mlp_in, dw_csgu, w_mlp_out, dw_merge, w_merge)
```

```python
import math

import jax
import jax.numpy as jnp
from jax import lax
import jax.experimental.pallas as pl
import jax.experimental.pallas.tpu as pltpu

F32 = jnp.float32
BF16 = jnp.bfloat16
LANES = 128
SUBL = 8
PAD = 8
XR = 16
EPS = 1e-5


def _dot(a, b):
    return jnp.dot(a, b, preferred_element_type=F32)


def _dot_nt(a, b):
    return lax.dot_general(a, b, (((1,), (1,)), ((), ())),
                           preferred_element_type=F32)


def _layernorm(v):
    mu = jnp.mean(v, axis=-1, keepdims=True)
    c = v - mu
    var = jnp.mean(c * c, axis=-1, keepdims=True)
    return c * lax.rsqrt(var + EPS)


def _gelu(v):
    c0 = math.sqrt(2.0 / math.pi)
    inner = v * (c0 + (c0 * 0.044715) * (v * v))
    half = 0.5 * v
    return half + half * jnp.tanh(inner)


def _rowmax(sc):
    cw = sc.shape[1]
    nfull = cw // LANES
    mr = None
    for t in range(nfull):
        st = sc[:, t * LANES:(t + 1) * LANES]
        mr = st if mr is None else jnp.maximum(mr, st)
    m = jnp.max(mr, axis=1, keepdims=True)
    if cw % LANES:
        m = jnp.maximum(m, jnp.max(sc[:, nfull * LANES:], axis=1, keepdims=True))
    return m


def _conv_rows(src, c, dw, r0, n):
    k_taps = dw.shape[0]
    half = k_taps // 2
    nv = n // SUBL
    w = src[c, pl.ds(r0, n + 2 * PAD), :].reshape(nv + 2, SUBL, LANES)
    sub = lax.broadcasted_iota(jnp.int32, (nv, SUBL, LANES), 1)
    acc = w[1:nv + 1] * dw[half:half + 1, :]
    for k in range(k_taps):
        off = k - half
        if off == 0:
            continue
        r = pltpu.roll(w, (-off) % SUBL, 1)
        if off > 0:
            t = jnp.where(sub < SUBL - off, r[1:nv + 1], r[2:nv + 2])
        else:
            t = jnp.where(sub >= -off, r[1:nv + 1], r[0:nv])
        acc = acc + t * dw[k:k + 1, :]
    return acc.reshape(n, LANES)


def _make_kernel(B, T, D, TQ, K, CK):
    NT = T // TQ
    NC = D // LANES
    HALF = K // 2
    YR = TQ - XR
    chunks = [(c0, min(CK, T - c0)) for c0 in range(0, T, CK)]
    NCH = len(chunks)
    PU = 3
    assert (NT - 1) % PU == 0 and NCH == 8 and HALF <= PAD
    qk_scale = (D ** -0.5) * math.log2(math.e)

    def kernel(x_hbm, wqkv_hbm, wao_hbm, win_hbm, dwc_hbm, wout_hbm,
               dwm_hbm, wmg_hbm, o_hbm,
               x_s, wqkv_ref, wao_ref, win_ref, dwc_ref, wout_ref, dwm_ref,
               wmg_ref, o_s,
               wqk_s, wvo_s, xa_s, xv_s, q_s, u_s, gn_s, mg_s, ml_s,
               xsem, wsem, osem):

        def x_copy(b, j):
            rows = pl.ds(pl.multiple_of(j * TQ, 16), TQ)
            return pltpu.make_async_copy(x_hbm.at[b, rows], x_s.at[b, rows],
                                         xsem.at[b * NT + j])

        def w_copy(k, src, dst):
            return pltpu.make_async_copy(src, dst, wsem.at[k])

        cp_wqk = w_copy(0, wqkv_hbm.at[:, 0:2 * D], wqkv_ref.at[:, 0:2 * D])
        cp_win = w_copy(1, win_hbm, win_ref)
        late_copies = [
            w_copy(2, wqkv_hbm.at[:, 2 * D:3 * D], wqkv_ref.at[:, 2 * D:3 * D]),
            w_copy(3, wao_hbm, wao_ref), w_copy(4, dwc_hbm, dwc_ref),
            w_copy(5, wout_hbm, wout_ref), w_copy(6, dwm_hbm, dwm_ref),
            w_copy(7, wmg_hbm, wmg_ref)]

        def lag_pos(n):
            e = n * TQ - XR
            b = e // T
            return b, pl.multiple_of(e - b * T, 16)

        def o_lag_copy(n):
            b, r = lag_pos(n)
            slot = lax.rem(n, 2)
            return pltpu.make_async_copy(
                o_s.at[slot, pl.ds(0, XR)], o_hbm.at[b, pl.ds(r, XR)],
                osem.at[2 * slot])

        def o_main_copy(n):
            b = n // NT
            r = pl.multiple_of((n - b * NT) * TQ, 16)
            slot = lax.rem(n, 2)
            return pltpu.make_async_copy(
                o_s.at[slot, pl.ds(XR, YR)], o_hbm.at[b, pl.ds(r, YR)],
                osem.at[2 * slot + 1])

        x_copy(0, 0).start()
        cp_wqk.start()

        zrow = jnp.zeros((PAD, LANES), F32)
        for c in range(NC):
            gn_s[c, 0:PAD, :] = zrow
            gn_s[c, PAD + T:PAD + T + PAD, :] = zrow
        ztail = jnp.zeros((XR + 2 * PAD, LANES), F32)
        for ref in (mg_s, ml_s):
            for c in range(NC):
                ref[c, 0:PAD, :] = zrow
                ref[c, T - XR:T + 2 * PAD, :] = ztail

        cp_wqk.wait()
        cp_win.start()
        for u in range(PU):
            x_copy(0, 1 + u).start()
        wqk = _dot_nt(wqkv_ref[:, 0:D], wqkv_ref[:, D:2 * D]) * qk_scale
        wqk_s[...] = wqk.astype(BF16)

        def fold_vo():
            for cp in late_copies:
                cp.wait()
            wvo = _dot(wqkv_ref[:, 2 * D:3 * D], wao_ref[...])
            wvo_s[...] = (wvo - wvo[D - 1:D, :]).astype(BF16)

        def p1_norm(b, j):
            r0 = pl.multiple_of(j * TQ, 16)
            xn = _layernorm(x_s[b, pl.ds(r0, TQ), :].astype(F32))
            xa = xn.astype(BF16)
            xa_s[pl.ds(r0, TQ), :] = xa
            xv_s[pl.ds(r0, TQ), 0:D - LANES] = xa[:, 0:D - LANES]
            lane = lax.broadcasted_iota(jnp.int32, (TQ, LANES), 1)
            xv_s[pl.ds(r0, TQ), D - LANES:D] = jnp.where(
                lane == LANES - 1, 1.0, xn[:, D - LANES:D]).astype(BF16)
            q_s[pl.ds(r0, TQ), :] = _dot(xa, wqk_s[...]).astype(BF16)
            return xa

        def p1_mlp(j, xa=None):
            r0 = pl.multiple_of(j * TQ, 16)
            if xa is None:
                xa = xa_s[pl.ds(r0, TQ), :]
            g = _layernorm(_gelu(_dot(xa, win_ref[:, D:2 * D])))
            for c in range(NC):
                gn_s[c, pl.ds(PAD + r0, TQ), :] = g[:, c * LANES:(c + 1) * LANES]
            u_s[pl.ds(r0, TQ), :] = _dot(xa, win_ref[:, 0:D])

        def merge_weights():
            dwm = dwm_ref[...].astype(F32)
            row = lax.broadcasted_iota(jnp.int32, dwm.shape, 0)
            return jnp.where(row == HALF, dwm + 1.0, dwm)

        def block(b, i):
            n = b * NT + i
            r0 = pl.multiple_of(i * TQ, 16)
            rl = pl.multiple_of(jnp.where(i == 0, T, r0) - XR, 16)
            bl = jnp.maximum(jnp.where(i == 0, b - 1, b), 0)
            slot = lax.rem(n, 2)
            dwc = dwc_ref[...].astype(F32)
            dwm = merge_weights()
            state = {}

            def loc_chunk(c):
                cols = slice(c * LANES, (c + 1) * LANES)
                gc = _conv_rows(gn_s, c, dwc[:, cols], r0, TQ)
                t = (_gelu(u_s[pl.ds(r0, TQ), cols]) * gc).astype(BF16)
                o = _dot(t, wout_ref[cols, :])
                state["loc"] = o if c == 0 else state["loc"] + o
                if c == NC - 1:
                    for cc in range(NC):
                        ml_s[cc, pl.ds(PAD + r0, TQ), :] = (
                            state["loc"][:, cc * LANES:(cc + 1) * LANES])

            def mrg_chunk(c):
                cols = slice(c * LANES, (c + 1) * LANES)
                src = mg_s if c < NC else ml_s
                mm = jnp.concatenate(
                    [_conv_rows(src, c % NC, dwm[:, cols], rl, XR),
                     _conv_rows(src, c % NC, dwm[:, cols], r0, YR)], axis=0)
                o = _dot(mm.astype(BF16), wmg_ref[cols, :])
                state["y"] = o if "y" not in state else state["y"] + o
                state["ny"] = state.get("ny", 0) + 1
                if state["ny"] == 2 * NC:
                    y = state["y"]
                    o_s[slot, 0:XR, :] = (
                        x_s[bl, pl.ds(rl, XR), :].astype(F32) + y[0:XR]
                    ).astype(o_s.dtype)
                    o_s[slot, XR:TQ, :] = (
                        x_s[b, pl.ds(r0, YR), :].astype(F32) + y[XR:TQ]
                    ).astype(o_s.dtype)

            slots = [[], [(loc_chunk, 0)], [(loc_chunk, 1)], [(loc_chunk, 2)],
                     [(loc_chunk, 3)], [], [], [(mrg_chunk, 4), (mrg_chunk, 5)]]
            post = [6, 7, 0, 1, 2, 3]

            q = q_s[pl.ds(r0, TQ), :]

            def qk(idx):
                c0, cw = chunks[idx]
                return _dot_nt(q, xa_s[c0:c0 + cw, :])

            nxt = qk(0)
            acc = None
            m = None
            for idx, (c0, cw) in enumerate(chunks):
                sc = nxt
                if idx + 1 < NCH:
                    nxt = qk(idx + 1)
                mc = _rowmax(sc)
                mn = mc if m is None else jnp.maximum(m, mc)
                p = jnp.exp2(sc - mn).astype(BF16)
                o = _dot(p, xv_s[c0:c0 + cw, :])
                acc = o if acc is None else acc * jnp.exp2(m - mn) + o
                m = mn
                for f, c in slots[idx]:
                    f(c)
            on = (acc * (1.0 / acc[:, D - 1:D])).astype(BF16)
            glob = _dot(on, wvo_s[...])
            for c in range(NC):
                mg_s[c, pl.ds(PAD + r0, TQ), :] = glob[:, c * LANES:(c + 1) * LANES]
            for c in post:
                mrg_chunk(c)

            o_main_copy(n).start()

            @pl.when(n >= 1)
            def _():
                o_lag_copy(n).start()
                o_main_copy(n - 1).wait()

            @pl.when(n >= 2)
            def _():
                o_lag_copy(n - 1).wait()

        def batch_body(b, carry):
            x_copy(b, 0).wait()
            p1_norm(b, 0)
            pl.when(b == 0)(cp_win.wait)

            def p1_body(jj, c):
                j0 = 1 + jj * PU

                @pl.when(jnp.logical_and(b == 0, j0 + PU < NT))
                def _():
                    for u in range(PU):
                        x_copy(0, j0 + PU + u).start()

                @pl.when(jnp.logical_and(b == 0, jj == 1))
                def _():
                    for cp in late_copies:
                        cp.start()
                for u in range(PU):
                    x_copy(b, j0 + u).wait()
                xa = None
                for u in range(PU):
                    p1_mlp(j0 + u - 1, xa)
                    xa = p1_norm(b, j0 + u)
                return c
            lax.fori_loop(0, (NT - 1) // PU, p1_body, 0)
            p1_mlp(NT - 1)
            pl.when(b == 0)(fold_vo)

            def att_body(i, c):
                block(b, i)

                @pl.when(b + 1 < B)
                def _():
                    x_copy(b + 1, i).start()
                return c
            lax.fori_loop(0, NT, att_body, 0)
            return carry

        lax.fori_loop(0, B, batch_body, 0)

        nl = B * NT
        dwm = merge_weights()
        y = None
        for c in range(2 * NC):
            cols = slice(c * LANES, (c + 1) * LANES)
            src = mg_s if c < NC else ml_s
            mm = _conv_rows(src, c % NC, dwm[:, cols], T - XR, XR)
            o = _dot(mm.astype(BF16), wmg_ref[cols, :])
            y = o if y is None else y + o
        o_s[nl % 2, 0:XR, :] = (
            x_s[B - 1, T - XR:T, :].astype(F32) + y).astype(o_s.dtype)
        o_lag_copy(nl).start()
        o_lag_copy(nl - 1).wait()
        o_main_copy(nl - 1).wait()
        o_lag_copy(nl).wait()

    return kernel


@jax.jit
def pallas_standalone__conformer_family_e_branchformer__speech_kernel(
    x, w_qkv, w_att_out, w_mlp_in, dw_csgu, w_mlp_out, dw_merge, w_merge,
):
    B, T, D = x.shape
    K = dw_csgu.shape[0]
    TQ = 400
    CK = 512
    NT = T // TQ
    NC = D // LANES
    T2 = T + 2 * PAD
    dt = x.dtype
    hbm = pl.BlockSpec(memory_space=pl.ANY)
    return pl.pallas_call(
        _make_kernel(B, T, D, TQ, K, CK),
        in_specs=[hbm] * 8,
        out_specs=hbm,
        out_shape=jax.ShapeDtypeStruct((B, T, D), dt),
        scratch_shapes=[
            pltpu.VMEM((B, T, D), dt),
            pltpu.VMEM(w_qkv.shape, dt),
            pltpu.VMEM(w_att_out.shape, dt),
            pltpu.VMEM(w_mlp_in.shape, dt),
            pltpu.VMEM(dw_csgu.shape, dt),
            pltpu.VMEM(w_mlp_out.shape, dt),
            pltpu.VMEM(dw_merge.shape, dt),
            pltpu.VMEM(w_merge.shape, dt),
            pltpu.VMEM((2, TQ, D), dt),
            pltpu.VMEM((D, D), BF16),
            pltpu.VMEM((D, D), BF16),
            pltpu.VMEM((T, D), BF16),
            pltpu.VMEM((T, D), BF16),
            pltpu.VMEM((T, D), BF16),
            pltpu.VMEM((T, D), F32),
            pltpu.VMEM((NC, T2, LANES), F32),
            pltpu.VMEM((NC, T2, LANES), F32),
            pltpu.VMEM((NC, T2, LANES), F32),
            pltpu.SemaphoreType.DMA((B * NT,)),
            pltpu.SemaphoreType.DMA((8,)),
            pltpu.SemaphoreType.DMA((4,)),
        ],
        compiler_params=pltpu.CompilerParams(
            vmem_limit_bytes=110 * 1024 * 1024,
            disable_bounds_checks=True),
        name="ebranchformer",
    )(x, w_qkv, w_att_out, w_mlp_in, dw_csgu, w_mlp_out, dw_merge, w_merge)
```

```python
import math

import jax
import jax.numpy as jnp
from jax import lax
import jax.experimental.pallas as pl
import jax.experimental.pallas.tpu as pltpu

F32 = jnp.float32
BF16 = jnp.bfloat16
LANES = 128
SUBL = 8
PAD = 8
XR = 16
EPS = 1e-5


def _dot(a, b):
    return jnp.dot(a, b, preferred_element_type=F32)


def _dot_nt(a, b):
    return lax.dot_general(a, b, (((1,), (1,)), ((), ())),
                           preferred_element_type=F32)


def _layernorm(v):
    mu = jnp.mean(v, axis=-1, keepdims=True)
    c = v - mu
    var = jnp.mean(c * c, axis=-1, keepdims=True)
    return c * lax.rsqrt(var + EPS)


def _gelu(v):
    c0 = math.sqrt(2.0 / math.pi)
    inner = v * (c0 + (c0 * 0.044715) * (v * v))
    half = 0.5 * v
    return half + half * jnp.tanh(inner)


def _rowmax(sc):
    cw = sc.shape[1]
    nfull = cw // LANES
    mr = None
    for t in range(nfull):
        st = sc[:, t * LANES:(t + 1) * LANES]
        mr = st if mr is None else jnp.maximum(mr, st)
    if mr is None:
        return jnp.max(sc, axis=1, keepdims=True)
    m = jnp.max(mr, axis=1, keepdims=True)
    if cw % LANES:
        m = jnp.maximum(m, jnp.max(sc[:, nfull * LANES:], axis=1, keepdims=True))
    return m


def _conv_rows(src, c, dw, r0, n):
    k_taps = dw.shape[0]
    half = k_taps // 2
    nv = n // SUBL
    w = src[c, pl.ds(r0, n + 2 * PAD), :].reshape(nv + 2, SUBL, LANES)
    sub = lax.broadcasted_iota(jnp.int32, (nv, SUBL, LANES), 1)
    acc = w[1:nv + 1] * dw[half:half + 1, :]
    for k in range(k_taps):
        off = k - half
        if off == 0:
            continue
        r = pltpu.roll(w, (-off) % SUBL, 1)
        if off > 0:
            t = jnp.where(sub < SUBL - off, r[1:nv + 1], r[2:nv + 2])
        else:
            t = jnp.where(sub >= -off, r[1:nv + 1], r[0:nv])
        acc = acc + t * dw[k:k + 1, :]
    return acc.reshape(n, LANES)


def _make_kernel(B, T, D, TQ, K, CK):
    NT = T // TQ
    NC = D // LANES
    HALF = K // 2
    YR = TQ - XR
    rem = T % LANES
    full = T - rem
    chunks = [(full, rem)] + [(c0, min(CK, full - c0)) for c0 in range(0, full, CK)]
    NCH = len(chunks)
    PU = 3
    assert (NT - 1) % PU == 0 and NCH == 9 and HALF <= PAD
    qk_scale = (D ** -0.5) * math.log2(math.e)

    def kernel(x_hbm, wqkv_hbm, wao_hbm, win_hbm, dwc_hbm, wout_hbm,
               dwm_hbm, wmg_hbm, o_hbm,
               x_s, wqk_ref, wv_ref, wao_ref, win_ref, dwc_ref, wout_ref, dwm_ref,
               wmg_ref, o_s,
               wqk_s, wvo_s, xa_s, xv_s, q_s, u_s, gn_s, mg_s, ml_s,
               xsem, wsem, osem):

        def x_copy(b, j):
            rows = pl.ds(pl.multiple_of(j * TQ, 16), TQ)
            return pltpu.make_async_copy(x_hbm.at[b, rows], x_s.at[b * NT + j],
                                         xsem.at[b * NT + j])

        def w_copy(k, src, dst):
            return pltpu.make_async_copy(src, dst, wsem.at[k])

        cp_wqk = w_copy(0, wqkv_hbm.at[:, 0:2 * D], wqk_ref)
        cp_win = w_copy(1, win_hbm, win_ref)
        cp_wv = w_copy(2, wqkv_hbm.at[:, 2 * D:3 * D], wv_ref)
        cp_wao = w_copy(3, wao_hbm, wao_ref)
        late_copies = [
            w_copy(4, dwc_hbm, dwc_ref), w_copy(5, wout_hbm, wout_ref),
            w_copy(6, dwm_hbm, dwm_ref), w_copy(7, wmg_hbm, wmg_ref)]

        def lag_pos(n):
            e = n * TQ - XR
            b = e // T
            return b, pl.multiple_of(e - b * T, 16)

        def o_lag_copy(n):
            b, r = lag_pos(n)
            slot = lax.rem(n, 2)
            return pltpu.make_async_copy(
                o_s.at[slot, pl.ds(0, XR)], o_hbm.at[b, pl.ds(r, XR)],
                osem.at[2 * slot])

        def o_main_copy(n):
            b = n // NT
            r = pl.multiple_of((n - b * NT) * TQ, 16)
            slot = lax.rem(n, 2)
            return pltpu.make_async_copy(
                o_s.at[slot, pl.ds(XR, YR)], o_hbm.at[b, pl.ds(r, YR)],
                osem.at[2 * slot + 1])

        x_copy(0, 0).start()
        cp_wqk.start()
        cp_wv.start()
        cp_wao.start()
        cp_win.start()
        for u in range(PU):
            x_copy(0, 1 + u).start()

        zrow = jnp.zeros((PAD, LANES), F32)
        for c in range(NC):
            gn_s[c, 0:PAD, :] = zrow
            gn_s[c, PAD + T:PAD + T + PAD, :] = zrow
        ztail = jnp.zeros((XR + 2 * PAD, LANES), F32)
        for ref in (mg_s, ml_s):
            for c in range(NC):
                ref[c, 0:PAD, :] = zrow
                ref[c, T - XR:T + 2 * PAD, :] = ztail

        def ln_tile(b, j):
            r0 = pl.multiple_of(j * TQ, 16)
            xn = _layernorm(x_s[b * NT + j].astype(F32))
            xa = xn.astype(BF16)
            xa_s[pl.ds(r0, TQ), :] = xa
            xv_s[pl.ds(r0, TQ), 0:D - LANES] = xa[:, 0:D - LANES]
            lane = lax.broadcasted_iota(jnp.int32, (TQ, LANES), 1)
            xv_s[pl.ds(r0, TQ), D - LANES:D] = jnp.where(
                lane == LANES - 1, 1.0, xn[:, D - LANES:D]).astype(BF16)
            return xa

        x_copy(0, 0).wait()
        xa0 = ln_tile(0, 0)
        cp_wqk.wait()
        wqk = _dot_nt(wqk_ref[:, 0:D], wqk_ref[:, D:2 * D]) * qk_scale
        wqk = wqk.astype(BF16)
        wqk_s[...] = wqk
        q_s[0:TQ, :] = _dot(xa0, wqk).astype(BF16)

        cp_wv.wait()
        cp_wao.wait()
        wvo = _dot(wv_ref[...], wao_ref[...])
        wvo_s[...] = (wvo - wvo[D - 1:D, :]).astype(BF16)

        def wait_late():
            for cp in late_copies:
                cp.wait()

        def p1_norm(b, j, split=False):
            r0 = pl.multiple_of(j * TQ, 16)
            xa = ln_tile(b, j)
            if split:
                bounds = [0, 112, 208, 304, TQ]
                for lo, hi in zip(bounds[:-1], bounds[1:]):
                    q_s[pl.ds(r0 + lo, hi - lo), :] = _dot(
                        xa[lo:hi], wqk_s[...]).astype(BF16)
            else:
                q_s[pl.ds(r0, TQ), :] = _dot(xa, wqk_s[...]).astype(BF16)
            return xa

        def p1_mlp(j, xa=None):
            r0 = pl.multiple_of(j * TQ, 16)
            if xa is None:
                xa = xa_s[pl.ds(r0, TQ), :]
            gs = []
            for c in range(NC):
                cols = slice(c * LANES, (c + 1) * LANES)
                gs.append(_gelu(_dot(xa, win_ref[:, D + c * LANES:D + (c + 1) * LANES])))
                u_s[pl.ds(r0, TQ), cols] = _dot(xa, win_ref[:, cols])
            g = _layernorm(jnp.concatenate(gs, axis=1))
            for c in range(NC):
                gn_s[c, pl.ds(PAD + r0, TQ), :] = g[:, c * LANES:(c + 1) * LANES]

        def merge_weights():
            dwm = dwm_ref[...].astype(F32)
            row = lax.broadcasted_iota(jnp.int32, dwm.shape, 0)
            return jnp.where(row == HALF, dwm + 1.0, dwm)

        def block(b, i):
            n = b * NT + i
            r0 = pl.multiple_of(i * TQ, 16)
            rl = pl.multiple_of(jnp.where(i == 0, T, r0) - XR, 16)
            nl = jnp.maximum(n - 1, 0)
            slot = lax.rem(n, 2)
            dwc = dwc_ref[...].astype(F32)
            dwm = merge_weights()
            state = {}

            def loc_chunk(c):
                cols = slice(c * LANES, (c + 1) * LANES)
                gc = _conv_rows(gn_s, c, dwc[:, cols], r0, TQ)
                t = (_gelu(u_s[pl.ds(r0, TQ), cols]) * gc).astype(BF16)
                o = _dot(t, wout_ref[cols, :])
                state["loc"] = o if c == 0 else state["loc"] + o
                if c == NC - 1:
                    for cc in range(NC):
                        ml_s[cc, pl.ds(PAD + r0, TQ), :] = (
                            state["loc"][:, cc * LANES:(cc + 1) * LANES])

            def mrg_chunk(c):
                cols = slice(c * LANES, (c + 1) * LANES)
                src = mg_s if c < NC else ml_s
                mm = jnp.concatenate(
                    [_conv_rows(src, c % NC, dwm[:, cols], rl, XR),
                     _conv_rows(src, c % NC, dwm[:, cols], r0, YR)], axis=0)
                o = _dot(mm.astype(BF16), wmg_ref[cols, :])
                state["y"] = o if "y" not in state else state["y"] + o
                state["ny"] = state.get("ny", 0) + 1
                if state["ny"] == 2 * NC:
                    y = state["y"]
                    o_s[slot, 0:XR, :] = (
                        x_s[nl, YR:TQ, :].astype(F32) + y[0:XR]
                    ).astype(o_s.dtype)
                    o_s[slot, XR:TQ, :] = (
                        x_s[n, 0:YR, :].astype(F32) + y[XR:TQ]
                    ).astype(o_s.dtype)

            slots = [[], [], [(loc_chunk, 0)], [(loc_chunk, 1)], [(loc_chunk, 2)],
                     [(loc_chunk, 3)], [], [], [(mrg_chunk, 4), (mrg_chunk, 5)]]
            post = [6, 7, 0, 1, 2, 3]

            q = q_s[pl.ds(r0, TQ), :]

            def qk(idx):
                c0, cw = chunks[idx]
                return _dot_nt(q, xa_s[c0:c0 + cw, :])

            nxt = qk(0)
            acc = None
            m = None
            for idx, (c0, cw) in enumerate(chunks):
                sc = nxt
                if idx + 1 < NCH:
                    nxt = qk(idx + 1)
                mc = _rowmax(sc)
                mn = mc if m is None else jnp.maximum(m, mc)
                p = jnp.exp2(sc - mn).astype(BF16)
                o = _dot(p, xv_s[c0:c0 + cw, :])
                acc = o if acc is None else acc * jnp.exp2(m - mn) + o
                m = mn
                for f, c in slots[idx]:
                    f(c)
            on = (acc * (1.0 / acc[:, D - 1:D])).astype(BF16)
            glob = _dot(on, wvo_s[...])
            for c in range(NC):
                mg_s[c, pl.ds(PAD + r0, TQ), :] = glob[:, c * LANES:(c + 1) * LANES]
            for c in post:
                mrg_chunk(c)

            o_main_copy(n).start()

            @pl.when(n >= 1)
            def _():
                o_lag_copy(n).start()
                o_main_copy(n - 1).wait()

            @pl.when(n >= 2)
            def _():
                o_lag_copy(n - 1).wait()

        def batch_body(b, carry):
            @pl.when(b > 0)
            def _():
                x_copy(b, 0).wait()
                p1_norm(b, 0, split=True)
            pl.when(b == 0)(cp_win.wait)

            for u in range(PU):
                x_copy(b, 1 + u).wait()

            @pl.when(b == 0)
            def _():
                for u in range(PU):
                    x_copy(0, 1 + PU + u).start()

            def p1_body(jj, c):
                j0 = 1 + jj * PU
                xa = None
                for u in range(PU):
                    p1_mlp(j0 + u - 1, xa)
                    xa = p1_norm(b, j0 + u)

                @pl.when(jnp.logical_and(b == 0, jj == 0))
                def _():
                    for cp in late_copies:
                        cp.start()

                @pl.when(jnp.logical_and(b == 0, j0 + 2 * PU < NT))
                def _():
                    for u in range(PU):
                        x_copy(0, j0 + 2 * PU + u).start()

                @pl.when(j0 + PU < NT)
                def _():
                    for u in range(PU):
                        x_copy(b, j0 + PU + u).wait()
                return c
            lax.fori_loop(0, (NT - 1) // PU, p1_body, 0)
            p1_mlp(NT - 1)
            pl.when(b == 0)(wait_late)

            def att_body(i, c):
                block(b, i)

                @pl.when(b + 1 < B)
                def _():
                    x_copy(b + 1, i).start()
                return c
            lax.fori_loop(0, NT, att_body, 0)
            return carry

        lax.fori_loop(0, B, batch_body, 0)

        nl = B * NT
        dwm = merge_weights()
        y = None
        for c in range(2 * NC):
            cols = slice(c * LANES, (c + 1) * LANES)
            src = mg_s if c < NC else ml_s
            mm = _conv_rows(src, c % NC, dwm[:, cols], T - XR, XR)
            o = _dot(mm.astype(BF16), wmg_ref[cols, :])
            y = o if y is None else y + o
        o_s[nl % 2, 0:XR, :] = (
            x_s[B * NT - 1, YR:TQ, :].astype(F32) + y).astype(o_s.dtype)
        o_lag_copy(nl).start()
        o_lag_copy(nl - 1).wait()
        o_main_copy(nl - 1).wait()
        o_lag_copy(nl).wait()

    return kernel


@jax.jit
def pallas_standalone__conformer_family_e_branchformer__speech_kernel(
    x, w_qkv, w_att_out, w_mlp_in, dw_csgu, w_mlp_out, dw_merge, w_merge,
):
    B, T, D = x.shape
    K = dw_csgu.shape[0]
    TQ = 400
    CK = 512
    NT = T // TQ
    NC = D // LANES
    T2 = T + 2 * PAD
    dt = x.dtype
    hbm = pl.BlockSpec(memory_space=pl.ANY)
    return pl.pallas_call(
        _make_kernel(B, T, D, TQ, K, CK),
        in_specs=[hbm] * 8,
        out_specs=hbm,
        out_shape=jax.ShapeDtypeStruct((B, T, D), dt),
        scratch_shapes=[
            pltpu.VMEM((B * NT, TQ, D), dt),
            pltpu.VMEM((D, 2 * D), dt),
            pltpu.VMEM((D, D), dt),
            pltpu.VMEM(w_att_out.shape, dt),
            pltpu.VMEM(w_mlp_in.shape, dt),
            pltpu.VMEM(dw_csgu.shape, dt),
            pltpu.VMEM(w_mlp_out.shape, dt),
            pltpu.VMEM(dw_merge.shape, dt),
            pltpu.VMEM(w_merge.shape, dt),
            pltpu.VMEM((2, TQ, D), dt),
            pltpu.VMEM((D, D), BF16),
            pltpu.VMEM((D, D), BF16),
            pltpu.VMEM((T, D), BF16),
            pltpu.VMEM((T, D), BF16),
            pltpu.VMEM((T, D), BF16),
            pltpu.VMEM((T, D), F32),
            pltpu.VMEM((NC, T2, LANES), F32),
            pltpu.VMEM((NC, T2, LANES), F32),
            pltpu.VMEM((NC, T2, LANES), F32),
            pltpu.SemaphoreType.DMA((B * NT,)),
            pltpu.SemaphoreType.DMA((8,)),
            pltpu.SemaphoreType.DMA((4,)),
        ],
        compiler_params=pltpu.CompilerParams(
            vmem_limit_bytes=110 * 1024 * 1024,
            disable_bounds_checks=True),
        name="ebranchformer",
    )(x, w_qkv, w_att_out, w_mlp_in, dw_csgu, w_mlp_out, dw_merge, w_merge)
```
